```python
import os as _os
_os.environ.setdefault("JAX_PLATFORMS", "cpu")
import jax
import jax.numpy as jnp

def _softmax(x, axis=-1):
    return jax.nn.softmax(x, axis=axis)
def _gelu(x):
    return jax.nn.gelu(x, approximate=True)
def _silu(x):
    return jax.nn.silu(x)
def _sigmoid(x):
    return jax.nn.sigmoid(x)
def _layernorm(x, axis=-1, eps=1e-5):
    m = jnp.mean(x, axis=axis, keepdims=True)
    v = jnp.var(x, axis=axis, keepdims=True)
    return (x - m) / jnp.sqrt(v + eps)
def _scatter_add(tgt, idx, src, axis=0):
    return tgt.at[idx].add(src)
def _segment_sum(src, seg, n):
    return jax.ops.segment_sum(src, seg, n)
class _Rng:
    def __init__(self, key):
        self._k = key
    def _next(self):
        self._k, sub = jax.random.split(self._k)
        return sub
    def normal(self, shape):
        return jax.random.normal(self._next(), shape, dtype=jnp.bfloat16)
    def randint(self, lo, hi, shape):
        return jax.random.randint(self._next(), shape, lo, hi, dtype=jnp.int32)
    def uniform(self, shape, lo=0.0, hi=1.0):
        return jax.random.uniform(self._next(), shape, jnp.bfloat16, lo, hi)
    def permutation(self, n):
        return jax.random.permutation(self._next(), n)


kernel_name = 'parallel_sum__grouped_kv_mqa__dense_activation_silu__prompt'

def setup_inputs():
    _rng = _Rng(jax.random.key(int.from_bytes(__import__("os").urandom(4), "little")))
    _w = (lambda a: (lambda t: t.astype(jnp.bfloat16) if jnp.issubdtype(t.dtype, jnp.floating) else t)(jnp.asarray(a)))
    def _A_setup():
        B, S, D, H = 1, 2048, 512, 32
        Dh = D // H
        return {
            "x": _w((lambda *s: _rng.normal(s) * 0.05)(B, S, D)),
            "wq": _w((lambda *s: _rng.normal(s) * 0.05)(D, H * Dh)),
            "wk": _w((lambda *s: _rng.normal(s) * 0.05)(D, Dh)),
            "wv": _w((lambda *s: _rng.normal(s) * 0.05)(D, Dh)),
            "wo": _w((lambda *s: _rng.normal(s) * 0.05)(H * Dh, D)),
        }
    _A_in = _A_setup()

    def _B_setup():
        B, S, D, F = 1, 2048, 512, 1376
        return {
            "x": _w((lambda *s: _rng.normal(s) * 0.05)(B, S, D)),
            "w1": _w((lambda *s: _rng.normal(s) * 0.05)(D, F) * (D ** -0.5)),
            "w2": _w((lambda *s: _rng.normal(s) * 0.05)(F, D) * (F ** -0.5)),
        }
    _B_in = _B_setup()

    return {
        "A_x": _A_in["x"],
        "A_wq": _A_in["wq"],
        "A_wk": _A_in["wk"],
        "A_wv": _A_in["wv"],
        "A_wo": _A_in["wo"],
        "B_x": _B_in["x"],
        "B_w1": _B_in["w1"],
        "B_w2": _B_in["w2"],
    }

def reference(A_x, A_wq, A_wk, A_wv, A_wo, B_x, B_w1, B_w2):
    def _A_ref(x, wq, wk, wv, wo):
        B, S, D = x.shape
        H = 32
        Dh = D // H
        q = (lambda x, *d: x.transpose(*d))((x @ wq).reshape(B, S, H, Dh), 0, 2, 1, 3)
        k = x @ wk
        v = x @ wv
        scores = jnp.einsum("bhqd,bkd->bhqk", q, k) * (Dh ** -0.5)
        p = _softmax(scores, axis=-1)
        o = jnp.einsum("bhqk,bkd->bhqd", p, v)
        return (lambda x, *d: x.transpose(*d))(o, 0, 2, 1, 3).reshape(B, S, H * Dh) @ wo

    def _B_ref(x, w1, w2):
        h = jnp.einsum("bsd,df->bsf", x, w1)
        h = _silu(h)
        out = jnp.einsum("bsf,fd->bsd", h, w2)
        return out

    x = A_x
    xn = _layernorm(x, axis=-1)
    return x + _A_ref(xn, A_wq, A_wk, A_wv, A_wo) + _B_ref(xn, B_w1, B_w2)
```

```python
import math

import jax
import jax.numpy as jnp
import jax.experimental.pallas as pl
import jax.experimental.pallas.tpu as pltpu

_H = 32
_TQ = 512
_KC = 256
_NH = 2
_LAG = 1
_SAFE_BOUND = 40.0

_NT = (((1,), (1,)), ((), ()))
_TN = (((0,), (0,)), ((), ()))
_F32 = jnp.float32
_BF16 = jnp.bfloat16


def _dot(a, b, dims=None):
    if dims is None:
        return jnp.dot(a, b, preferred_element_type=_F32)
    return jax.lax.dot_general(a, b, dims, preferred_element_type=_F32)


def _kernel(x_ref, wq_ref, wk_ref, wv_ref, wo_ref, w1_ref, w2_ref, o_ref,
            xn_ref, wqt_ref, ka_ref, vt_ref, kmax_ref, qa_ref, ot_ref):
    S, D = x_ref.shape
    Dh = D // _H
    F = w1_ref.shape[1]
    step = pl.program_id(0)

    @pl.when(step == 0)
    def _prologue():
        def ln(i, c):
            r = pl.ds(pl.multiple_of(i * 256, 256), 256)
            x = x_ref[r, :].astype(_F32)
            m = jnp.mean(x, axis=-1, keepdims=True)
            xc = x - m
            v = jnp.mean(xc * xc, axis=-1, keepdims=True)
            xn_ref[r, :] = (xc / jnp.sqrt(v + 1e-5)).astype(_BF16)
            return c
        jax.lax.fori_loop(0, S // 256, ln, 0)
        wqt_ref[...] = wq_ref[...].astype(_F32).T.astype(_BF16)
        wkv = jnp.concatenate(
            [wk_ref[...].astype(_F32), wv_ref[...].astype(_F32),
             jnp.zeros((D, 128 - 2 * Dh), _F32)], axis=1)
        wkvt = wkv.T[:2 * Dh].astype(_BF16)
        kvt = _dot(wkvt, xn_ref[...], _NT).astype(_BF16)
        vt_ref[...] = kvt[Dh:]
        kt = kvt[:Dh].astype(_F32)
        k2 = jnp.max(jnp.sum(kt * kt, axis=0, keepdims=True), axis=1, keepdims=True)
        kmax_ref[...] = jnp.broadcast_to(jnp.sqrt(k2), kmax_ref.shape)
        row = jax.lax.broadcasted_iota(jnp.int32, (128 - Dh, S), 0)
        kta = jnp.concatenate([kt, jnp.where(row == 0, 1.0, 0.0).astype(_F32)], axis=0)
        ka_ref[...] = kta.T[:, :2 * Dh].astype(_BF16)

    rows = pl.ds(pl.multiple_of(step * _TQ, _TQ), _TQ)
    xn = xn_ref[rows, :]

    qt = (_dot(wqt_ref[...], xn, _NT) * (Dh ** -0.5 * math.log2(math.e))).astype(_BF16)
    qt3 = qt.reshape(_H, Dh, _TQ)
    qf = qt3.astype(_F32)
    bound = jnp.sqrt(jnp.sum(qf * qf, axis=1, keepdims=True)) * (
        kmax_ref[0:1, :].reshape(1, 1, _TQ) * (1.0 + 2.0 ** -6))
    row = jax.lax.broadcasted_iota(jnp.int32, (_H, Dh, _TQ), 1)
    qa_ref[:, :Dh, :] = qt3
    qa_ref[:, Dh:, :] = jnp.where(row == 0, -bound, 0.0).astype(_BF16)
    safe = jnp.max(bound) <= _SAFE_BOUND

    nc = S // _KC

    @pl.when(safe)
    def _fast():
        def body(i, c):
            work = [(h, c_) for h in range(_NH) for c_ in range(nc)]
            ps, acc, l = {}, {}, {}
            for t in range(len(work) + _LAG):
                if t < len(work):
                    h, cc = work[t]
                    p = jnp.exp2(_dot(ka_ref[cc * _KC:(cc + 1) * _KC, :], qa_ref[i * _NH + h]))
                    ls = jnp.sum(p.reshape(_KC // 8, 8, _TQ), axis=0)
                    l[h] = ls if cc == 0 else l[h] + ls
                    ps[t] = p.astype(_BF16)
                if t >= _LAG:
                    h, cc = work[t - _LAG]
                    o = _dot(vt_ref[:, cc * _KC:(cc + 1) * _KC], ps.pop(t - _LAG))
                    acc[h] = o if cc == 0 else acc[h] + o
                    if cc == nc - 1:
                        o = acc[h] / jnp.sum(l[h], axis=0, keepdims=True)
                        ot_ref[i * _NH + h] = o.astype(_BF16)
            return c
        jax.lax.fori_loop(0, _H // _NH, body, 0)

    @pl.when(jnp.logical_not(safe))
    def _exact():
        def body(h, c):
            s = _dot(ka_ref[:, :Dh], qa_ref[h, :Dh, :])
            p = jnp.exp2(s - jnp.max(s, axis=0, keepdims=True))
            o = _dot(vt_ref[...], p.astype(_BF16)) / jnp.sum(p, axis=0, keepdims=True)
            ot_ref[h] = o.astype(_BF16)
            return c
        jax.lax.fori_loop(0, _H, body, 0)

    out = x_ref[rows, :].astype(_F32) + _dot(ot_ref[...].reshape(D, _TQ), wo_ref[...], _TN)
    f0 = 0
    while f0 < F:
        f1 = min(f0 + 512, F)
        h = _dot(xn, w1_ref[:, f0:f1])
        a = (h / (1.0 + jnp.exp(-h))).astype(_BF16)
        out = out + _dot(a, w2_ref[f0:f1, :])
        f0 = f1
    o_ref[...] = out.astype(o_ref.dtype)


@jax.jit
def pallas_parallel_sum__grouped_kv_mqa__dense_activation_silu__prompt_kernel(
    A_x: jax.Array,
    A_wq: jax.Array,
    A_wk: jax.Array,
    A_wv: jax.Array,
    A_wo: jax.Array,
    B_x: jax.Array,
    B_w1: jax.Array,
    B_w2: jax.Array,
):
    del B_x
    B, S, D = A_x.shape
    assert B == 1
    Dh = D // _H
    full = lambda a: pl.BlockSpec(a.shape, lambda i: (0,) * a.ndim)
    args = (A_x.reshape(S, D), A_wq, A_wk, A_wv, A_wo, B_w1, B_w2)
    out = pl.pallas_call(
        _kernel,
        grid=(S // _TQ,),
        in_specs=[full(a) for a in args],
        out_specs=pl.BlockSpec((_TQ, D), lambda i: (i, 0)),
        out_shape=jax.ShapeDtypeStruct((S, D), A_x.dtype),
        scratch_shapes=[
            pltpu.VMEM((S, D), _BF16),
            pltpu.VMEM((D, D), _BF16),
            pltpu.VMEM((S, 2 * Dh), _BF16),
            pltpu.VMEM((Dh, S), _BF16),
            pltpu.VMEM((8, _TQ), _F32),
            pltpu.VMEM((_H, 2 * Dh, _TQ), _BF16),
            pltpu.VMEM((_H, Dh, _TQ), _BF16),
        ],
        compiler_params=pltpu.CompilerParams(
            dimension_semantics=("arbitrary",),
            vmem_limit_bytes=64 * 1024 * 1024,
        ),
    )(*args)
    return out.reshape(B, S, D)
```

```python
import math

import jax
import jax.numpy as jnp
import jax.experimental.pallas as pl
import jax.experimental.pallas.tpu as pltpu

_H = 32
_TQ = 512
_KC = 256
_NH = 2
_LAG = 1
_SAFE_BOUND = 40.0

_NT = (((1,), (1,)), ((), ()))
_TN = (((0,), (0,)), ((), ()))
_F32 = jnp.float32
_BF16 = jnp.bfloat16


def _dot(a, b, dims=None):
    if dims is None:
        return jnp.dot(a, b, preferred_element_type=_F32)
    return jax.lax.dot_general(a, b, dims, preferred_element_type=_F32)


def _kernel(x_ref, wq_ref, wk_ref, wv_ref, wo_ref, w1_ref, w2_ref, o_ref,
            xn_ref, wqt_ref, ka_ref, vt_ref, kmax_ref, qa_ref, ot_ref):
    S, D = x_ref.shape
    Dh = D // _H
    F = w1_ref.shape[0]
    step = pl.program_id(0)

    @pl.when(step == 0)
    def _prologue():
        def ln(i, c):
            r = pl.ds(pl.multiple_of(i * 256, 256), 256)
            x = x_ref[r, :].astype(_F32)
            m = jnp.mean(x, axis=-1, keepdims=True)
            xc = x - m
            v = jnp.mean(xc * xc, axis=-1, keepdims=True)
            xn_ref[r, :] = (xc / jnp.sqrt(v + 1e-5)).astype(_BF16)
            return c
        jax.lax.fori_loop(0, S // 256, ln, 0)
        wqt_ref[...] = wq_ref[...].astype(_F32).T.astype(_BF16)
        wkvt = jnp.concatenate([wk_ref[...], wv_ref[...]], axis=0)
        kvt = _dot(wkvt, xn_ref[...], _NT).astype(_BF16)
        vt_ref[...] = kvt[Dh:]
        kt = kvt[:Dh].astype(_F32)
        k2 = jnp.max(jnp.sum(kt * kt, axis=0, keepdims=True), axis=1, keepdims=True)
        kmax_ref[...] = jnp.broadcast_to(jnp.sqrt(k2), kmax_ref.shape)
        row = jax.lax.broadcasted_iota(jnp.int32, (128 - Dh, S), 0)
        kta = jnp.concatenate([kt, jnp.where(row == 0, 1.0, 0.0).astype(_F32)], axis=0)
        ka_ref[...] = kta.T[:, :2 * Dh].astype(_BF16)

    rows = pl.ds(pl.multiple_of(step * _TQ, _TQ), _TQ)
    xn = xn_ref[rows, :]

    qt = (_dot(wqt_ref[...], xn, _NT) * (Dh ** -0.5 * math.log2(math.e))).astype(_BF16)
    qt3 = qt.reshape(_H, Dh, _TQ)
    qf = qt3.astype(_F32)
    bound = jnp.sqrt(jnp.sum(qf * qf, axis=1, keepdims=True)) * (
        kmax_ref[0:1, :].reshape(1, 1, _TQ) * (1.0 + 2.0 ** -6))
    row = jax.lax.broadcasted_iota(jnp.int32, (_H, Dh, _TQ), 1)
    qa_ref[:, :Dh, :] = qt3
    qa_ref[:, Dh:, :] = jnp.where(row == 0, -bound, 0.0).astype(_BF16)
    safe = jnp.max(bound) <= _SAFE_BOUND

    nc = S // _KC

    @pl.when(safe)
    def _fast():
        def body(i, c):
            work = [(h, c_) for h in range(_NH) for c_ in range(nc)]
            ps, acc, l = {}, {}, {}
            for t in range(len(work) + _LAG):
                if t < len(work):
                    h, cc = work[t]
                    p = jnp.exp2(_dot(ka_ref[cc * _KC:(cc + 1) * _KC, :], qa_ref[i * _NH + h]))
                    ls = jnp.sum(p.reshape(_KC // 8, 8, _TQ), axis=0)
                    l[h] = ls if cc == 0 else l[h] + ls
                    ps[t] = p.astype(_BF16)
                if t >= _LAG:
                    h, cc = work[t - _LAG]
                    o = _dot(vt_ref[:, cc * _KC:(cc + 1) * _KC], ps.pop(t - _LAG))
                    acc[h] = o if cc == 0 else acc[h] + o
                    if cc == nc - 1:
                        o = acc[h] / jnp.sum(l[h], axis=0, keepdims=True)
                        ot_ref[i * _NH + h] = o.astype(_BF16)
            return c
        jax.lax.fori_loop(0, _H // _NH, body, 0)

    @pl.when(jnp.logical_not(safe))
    def _exact():
        def body(h, c):
            s = _dot(ka_ref[:, :Dh], qa_ref[h, :Dh, :])
            p = jnp.exp2(s - jnp.max(s, axis=0, keepdims=True))
            o = _dot(vt_ref[...], p.astype(_BF16)) / jnp.sum(p, axis=0, keepdims=True)
            ot_ref[h] = o.astype(_BF16)
            return c
        jax.lax.fori_loop(0, _H, body, 0)

    out = x_ref[rows, :].astype(_F32) + _dot(ot_ref[...].reshape(D, _TQ), wo_ref[...], _TN)
    f0 = 0
    while f0 < F:
        f1 = min(f0 + 512, F)
        h = _dot(xn, w1_ref[f0:f1, :], _NT)
        a = (h / (1.0 + jnp.exp(-h))).astype(_BF16)
        out = out + _dot(a, w2_ref[f0:f1, :])
        f0 = f1
    o_ref[...] = out.astype(o_ref.dtype)


@jax.jit
def pallas_parallel_sum__grouped_kv_mqa__dense_activation_silu__prompt_kernel(
    A_x: jax.Array,
    A_wq: jax.Array,
    A_wk: jax.Array,
    A_wv: jax.Array,
    A_wo: jax.Array,
    B_x: jax.Array,
    B_w1: jax.Array,
    B_w2: jax.Array,
):
    del B_x
    B, S, D = A_x.shape
    assert B == 1
    Dh = D // _H
    full = lambda a: pl.BlockSpec(a.shape, lambda i: (0,) * a.ndim)
    args = (A_x.reshape(S, D), A_wq, A_wk.T, A_wv.T, A_wo, B_w1.T, B_w2)
    out = pl.pallas_call(
        _kernel,
        grid=(S // _TQ,),
        in_specs=[full(a) for a in args],
        out_specs=pl.BlockSpec((_TQ, D), lambda i: (i, 0)),
        out_shape=jax.ShapeDtypeStruct((S, D), A_x.dtype),
        scratch_shapes=[
            pltpu.VMEM((S, D), _BF16),
            pltpu.VMEM((D, D), _BF16),
            pltpu.VMEM((S, 2 * Dh), _BF16),
            pltpu.VMEM((Dh, S), _BF16),
            pltpu.VMEM((8, _TQ), _F32),
            pltpu.VMEM((_H, 2 * Dh, _TQ), _BF16),
            pltpu.VMEM((_H, Dh, _TQ), _BF16),
        ],
        compiler_params=pltpu.CompilerParams(
            dimension_semantics=("arbitrary",),
            vmem_limit_bytes=64 * 1024 * 1024,
        ),
    )(*args)
    return out.reshape(B, S, D)
```

```python
import math

import jax
import jax.numpy as jnp
import jax.experimental.pallas as pl
import jax.experimental.pallas.tpu as pltpu

_H = 32
_TQ = 512
_KC = 128
_XC = 512
_FC = 512
_NH = 16
_LAG = 2
_SAFE_BOUND = 40.0

_NT = (((1,), (1,)), ((), ()))
_TN = (((0,), (0,)), ((), ()))
_F32 = jnp.float32
_BF16 = jnp.bfloat16


def _dot(a, b, dims=None):
    if dims is None:
        return jnp.dot(a, b, preferred_element_type=_F32)
    return jax.lax.dot_general(a, b, dims, preferred_element_type=_F32)


def _kernel(x_hbm, wq_hbm, wk_ref, wv_ref, wo_hbm, w1_hbm, w2_hbm, o_ref,
            x_ref, wq_ref, wo_ref, w1_ref, w2_ref, sems,
            xn_ref, wqt_ref, kt_ref, ka_ref, vt_ref, kmax_ref, qa_ref, ot_ref):
    S, D = x_ref.shape
    Dh = D // _H
    F = w1_ref.shape[0]
    step = pl.program_id(0)

    def x_copy(r, i):
        return pltpu.make_async_copy(x_hbm.at[r, :], x_ref.at[r, :], sems.at[i])

    nx = S // _XC
    wq_copy = pltpu.make_async_copy(wq_hbm, wq_ref, sems.at[nx])
    late = [pltpu.make_async_copy(src, dst, sems.at[nx + 1 + n]) for n, (src, dst) in
            enumerate(((wo_hbm, wo_ref), (w1_hbm, w1_ref), (w2_hbm, w2_ref)))]

    @pl.when(step == 0)
    def _prologue():
        for i in range(nx):
            x_copy(pl.ds(i * _XC, _XC), i).start()
        wq_copy.start()
        wkvt = jnp.concatenate([wk_ref[...], wv_ref[...]], axis=0)

        def ln(i, c):
            r = pl.ds(pl.multiple_of(i * _XC, _XC), _XC)
            x_copy(r, i).wait()
            x = x_ref[r, :].astype(_F32)
            m = jnp.mean(x, axis=-1, keepdims=True)
            xc = x - m
            v = jnp.mean(xc * xc, axis=-1, keepdims=True)
            xn = (xc / jnp.sqrt(v + 1e-5)).astype(_BF16)
            xn_ref[r, :] = xn
            kvt = _dot(wkvt, xn, _NT).astype(_BF16)
            kt_ref[:, r] = kvt[:Dh].astype(_F32)
            vt_ref[:, r] = kvt[Dh:]
            return c
        jax.lax.fori_loop(0, nx, ln, 0)
        for c in late:
            c.start()
        kt = kt_ref[...]
        k2 = jnp.max(jnp.sum(kt * kt, axis=0, keepdims=True), axis=1, keepdims=True)
        kmax_ref[...] = jnp.broadcast_to(jnp.sqrt(k2), kmax_ref.shape)
        row = jax.lax.broadcasted_iota(jnp.int32, (128 - Dh, S), 0)
        kta = jnp.concatenate([kt, jnp.where(row == 0, 1.0, 0.0).astype(_F32)], axis=0)
        ka_ref[...] = kta.T[:, :2 * Dh].astype(_BF16)
        wq_copy.wait()
        wqt_ref[...] = wq_ref[...].astype(_F32).T.astype(_BF16)

    rows = pl.ds(pl.multiple_of(step * _TQ, _TQ), _TQ)
    xn = xn_ref[rows, :]

    qt = (_dot(wqt_ref[...], xn, _NT) * (Dh ** -0.5 * math.log2(math.e))).astype(_BF16)

    qt3 = qt.reshape(_H, Dh, _TQ)
    qf = qt3.astype(_F32)
    bound = jnp.sqrt(jnp.sum(qf * qf, axis=1, keepdims=True)) * (
        kmax_ref[0:1, :].reshape(1, 1, _TQ) * (1.0 + 2.0 ** -6))
    row = jax.lax.broadcasted_iota(jnp.int32, (_H, Dh, _TQ), 1)
    qa_ref[:, :Dh, :] = qt3
    qa_ref[:, Dh:, :] = jnp.where(row == 0, -bound, 0.0).astype(_BF16)
    safe = jnp.max(bound) <= _SAFE_BOUND

    nc = S // _KC

    @pl.when(safe)
    def _fast():
        def body(i, c):
            work = [(h, c_) for h in range(_NH) for c_ in range(nc)]
            ps, acc, l = {}, {}, {}
            for t in range(len(work) + _LAG):
                if t < len(work):
                    h, cc = work[t]
                    p = jnp.exp2(_dot(ka_ref[cc * _KC:(cc + 1) * _KC, :], qa_ref[i * _NH + h]))
                    ls = jnp.sum(p.reshape(_KC // 8, 8, _TQ), axis=0)
                    l[h] = ls if cc == 0 else l[h] + ls
                    ps[t] = p.astype(_BF16)
                if t >= _LAG:
                    h, cc = work[t - _LAG]
                    o = _dot(vt_ref[:, cc * _KC:(cc + 1) * _KC], ps.pop(t - _LAG))
                    acc[h] = o if cc == 0 else acc[h] + o
                    if cc == nc - 1:
                        o = acc[h] / jnp.sum(l[h], axis=0, keepdims=True)
                        ot_ref[i * _NH + h] = o.astype(_BF16)
            return c
        jax.lax.fori_loop(0, _H // _NH, body, 0)

    @pl.when(jnp.logical_not(safe))
    def _exact():
        def body(h, c):
            s = _dot(ka_ref[:, :Dh], qa_ref[h, :Dh, :])
            p = jnp.exp2(s - jnp.max(s, axis=0, keepdims=True))
            o = _dot(vt_ref[...], p.astype(_BF16)) / jnp.sum(p, axis=0, keepdims=True)
            ot_ref[h] = o.astype(_BF16)
            return c
        jax.lax.fori_loop(0, _H, body, 0)

    @pl.when(step == 0)
    def _():
        for c in late:
            c.wait()

    fs = [(f0, min(f0 + _FC, F)) for f0 in range(0, F, _FC)]
    out = x_ref[rows, :].astype(_F32) + _dot(ot_ref[...].reshape(D, _TQ), wo_ref[...], _TN)
    act = None
    for j in range(len(fs) + 1):
        prev = act
        if j < len(fs):
            h = _dot(xn, w1_ref[fs[j][0]:fs[j][1], :], _NT)
            act = (h / (1.0 + jnp.exp(-h))).astype(_BF16)
        if j > 0:
            out = out + _dot(prev, w2_ref[fs[j - 1][0]:fs[j - 1][1], :])
    o_ref[...] = out.astype(o_ref.dtype)


@jax.jit
def pallas_parallel_sum__grouped_kv_mqa__dense_activation_silu__prompt_kernel(
    A_x: jax.Array,
    A_wq: jax.Array,
    A_wk: jax.Array,
    A_wv: jax.Array,
    A_wo: jax.Array,
    B_x: jax.Array,
    B_w1: jax.Array,
    B_w2: jax.Array,
):
    del B_x
    B, S, D = A_x.shape
    assert B == 1
    Dh = D // _H
    full = lambda a: pl.BlockSpec(a.shape, lambda i: (0,) * a.ndim)
    args = (A_x.reshape(S, D), A_wq, A_wk.T, A_wv.T, A_wo, B_w1.T, B_w2)
    out = pl.pallas_call(
        _kernel,
        grid=(S // _TQ,),
        in_specs=[full(a) if n in (2, 3) else pl.BlockSpec(memory_space=pl.ANY)
                  for n, a in enumerate(args)],
        out_specs=pl.BlockSpec((_TQ, D), lambda i: (i, 0)),
        out_shape=jax.ShapeDtypeStruct((S, D), A_x.dtype),
        scratch_shapes=[
            *(pltpu.VMEM(args[n].shape, args[n].dtype) for n in (0, 1, 4, 5, 6)),
            pltpu.SemaphoreType.DMA((S // _XC + 4,)),
            pltpu.VMEM((S, D), _BF16),
            pltpu.VMEM((D, D), _BF16),
            pltpu.VMEM((Dh, S), _F32),
            pltpu.VMEM((S, 2 * Dh), _BF16),
            pltpu.VMEM((Dh, S), _BF16),
            pltpu.VMEM((8, _TQ), _F32),
            pltpu.VMEM((_H, 2 * Dh, _TQ), _BF16),
            pltpu.VMEM((_H, Dh, _TQ), _BF16),
        ],
        compiler_params=pltpu.CompilerParams(
            dimension_semantics=("arbitrary",),
            vmem_limit_bytes=64 * 1024 * 1024,
        ),
    )(*args)
    return out.reshape(B, S, D)
```
